```python
import os as _os
_os.environ.setdefault("JAX_PLATFORMS", "cpu")
import jax
import jax.numpy as jnp

def _softmax(x, axis=-1):
    return jax.nn.softmax(x, axis=axis)
def _gelu(x):
    return jax.nn.gelu(x, approximate=True)
def _silu(x):
    return jax.nn.silu(x)
def _sigmoid(x):
    return jax.nn.sigmoid(x)
def _layernorm(x, axis=-1, eps=1e-5):
    m = jnp.mean(x, axis=axis, keepdims=True)
    v = jnp.var(x, axis=axis, keepdims=True)
    return (x - m) / jnp.sqrt(v + eps)
def _scatter_add(tgt, idx, src, axis=0):
    return tgt.at[idx].add(src)
def _segment_sum(src, seg, n):
    return jax.ops.segment_sum(src, seg, n)
class _Rng:
    def __init__(self, key):
        self._k = key
    def _next(self):
        self._k, sub = jax.random.split(self._k)
        return sub
    def normal(self, shape):
        return jax.random.normal(self._next(), shape, dtype=jnp.bfloat16)
    def randint(self, lo, hi, shape):
        return jax.random.randint(self._next(), shape, lo, hi, dtype=jnp.int32)
    def uniform(self, shape, lo=0.0, hi=1.0):
        return jax.random.uniform(self._next(), shape, jnp.bfloat16, lo, hi)
    def permutation(self, n):
        return jax.random.permutation(self._next(), n)


kernel_name = 'sequential_preLN__sliding_local_dilated__mixer_s_mlp__prompt'

def setup_inputs():
    _rng = _Rng(jax.random.key(int.from_bytes(__import__("os").urandom(4), "little")))
    _w = (lambda a: (lambda t: t.astype(jnp.bfloat16) if jnp.issubdtype(t.dtype, jnp.floating) else t)(jnp.asarray(a)))
    def _A_setup():
        B, S, D = 1, 2048, 448
        return {
            "x": _w((lambda *s: _rng.normal(s) * 0.05)(B, S, D)),
            "wqkv": _w((lambda *s: _rng.normal(s) * 0.05)(D, 3 * D)),
            "wo": _w((lambda *s: _rng.normal(s) * 0.05)(D, D)),
        }
    _A_in = _A_setup()

    def _B_setup():
        B, S, D, F = 1, 2048, 448, 1792
        return {
            "x":  _w((lambda *s: _rng.normal(s) * 0.05)(B, S, D)),
            "w1": _w((lambda *s: _rng.normal(s) * 0.8)(D, D) * (D ** -0.5)),
            "w2": _w((lambda *s: _rng.normal(s) * 0.8)(D, D) * (D ** -0.5)),
            "w3": _w((lambda *s: _rng.normal(s) * 0.8)(D, F) * (D ** -0.5)),
            "w4": _w((lambda *s: _rng.normal(s) * 0.8)(F, D) * (F ** -0.5)),
        }
    _B_in = _B_setup()

    return {
        "A_x": _A_in["x"],
        "A_wqkv": _A_in["wqkv"],
        "A_wo": _A_in["wo"],
        "B_x": _B_in["x"],
        "B_w1": _B_in["w1"],
        "B_w2": _B_in["w2"],
        "B_w3": _B_in["w3"],
        "B_w4": _B_in["w4"],
    }

def reference(A_x, A_wqkv, A_wo, B_x, B_w1, B_w2, B_w3, B_w4):
    def _A_ref(x, wqkv, wo):
        B, S, D = x.shape
        H = 16; Dh = D // H
        W, dil = 8, 2
        qkv = (lambda x, *d: x.transpose(*d))((x @ wqkv).reshape(B, S, 3, H, Dh), 2, 0, 3, 1, 4)
        q, k, v = qkv[0], qkv[1], qkv[2]
        scale = Dh ** -0.5
        pos = jnp.arange(S)
        off = jnp.arange(W) * dil
        idx = pos[:, None] - off[None, :]
        mask = idx >= 0
        idx_c = jnp.where(mask, idx, 0).reshape(-1)
        kg = k[:, :, idx_c, :].reshape(B, H, S, W, Dh)
        vg = v[:, :, idx_c, :].reshape(B, H, S, W, Dh)
        logits = jnp.einsum("bhsd,bhswd->bhsw", q, kg) * scale
        logits = jnp.where(mask[None, None, :, :], logits, -1e9)
        attn = _softmax(logits, axis=-1)
        o = jnp.einsum("bhsw,bhswd->bhsd", attn, vg)
        return (lambda x, *d: x.transpose(*d))(o, 0, 2, 1, 3).reshape(B, S, D) @ wo

    def _B_ref(x, w1, w2, w3, w4):
        B, S, D = x.shape
        h = _gelu(_layernorm(x, axis=-1) @ w1)
        c = D // 4
        g0 = jnp.pad(h[:, :, 0*c:1*c], ((0, 0), (1, 0), (0, 0)))[:, :S, :]
        g1 = jnp.pad(h[:, :, 1*c:2*c], ((0, 0), (0, 1), (0, 0)))[:, 1:, :]
        g2 = jnp.pad(h[:, :, 2*c:3*c], ((0, 0), (2, 0), (0, 0)))[:, :S, :]
        g3 = jnp.pad(h[:, :, 3*c:   ], ((0, 0), (0, 2), (0, 0)))[:, 2:, :]
        hs = jnp.concatenate([g0, g1, g2, g3], axis=-1) @ w2
        x1 = x + hs
        h2 = _gelu(_layernorm(x1, axis=-1) @ w3) @ w4
        return x1 + h2

    x = A_x
    h = x + _A_ref(_layernorm(x, axis=-1), A_wqkv, A_wo)
    h2 = h + _B_ref(_layernorm(h, axis=-1), B_w1, B_w2, B_w3, B_w4)
    return h2
```

```python
import functools
import jax
import jax.numpy as jnp
from jax import lax
import jax.experimental.pallas as pl
import jax.experimental.pallas.tpu as pltpu

S, D, H, DH, W, DIL, F = 2048, 448, 16, 28, 8, 2, 1792
TL = 256
NT = S // TL
NCB = TL // 128
NB = S // 128
EPS = 1e-5
LOG2E = 1.4426950408889634
QSCALE = (DH ** -0.5) * LOG2E
NEG = -1e9 * (DH ** 0.5)
DG = 1
F32, BF16, U32 = jnp.float32, jnp.bfloat16, jnp.uint32
KCH = [(0, 128), (128, 128), (256, 128), (384, 64)]
QCH = [(0, 512), (512, 512), (1024, 320)]


def _ln(x, scale=None):
    m = jnp.sum(x, axis=0, keepdims=True) * (1.0 / D)
    xc = x - m
    v = jnp.sum(xc * xc, axis=0, keepdims=True) * (1.0 / D)
    r = lax.rsqrt(v + EPS)
    if scale is not None:
        r = r * scale
    return xc * r


def _gelu_half(hx):
    c0 = 2.0 * 0.7978845608028654
    c1 = 8.0 * 0.7978845608028654 * 0.044715
    t = jnp.tanh(hx * (c0 + c1 * (hx * hx)))
    return hx + hx * t


def _dot(a, b):
    return jnp.dot(a, b, preferred_element_type=F32)


def _pk(x_bf16):
    return pltpu.bitcast(x_bf16, U32)


def _upk(x_u32):
    return pltpu.bitcast(x_u32, BF16)


def _kernel(x_hbm, wqkv_hbm, wo_hbm, w1_hbm, w2_hbm, w3_hbm, w4t_hbm, out_hbm,
            x_v, o_v, wqkv_v, wo_v, w1_v, w2_v, w3_v, w4_v,
            wqkvt, wot, w1t, w2t, w3t, tp, tp2,
            sem_w, sem_x, sem_o, sem_b):
    cp_qkv = [None] + [pltpu.make_async_copy(wqkv_hbm.at[:, pl.ds(c, n)], wqkv_v.at[:, pl.ds(c, n)], sem_w.at[j])
                       for j, (c, n) in enumerate(QCH[1:])]
    cp_a = [pltpu.make_async_copy(wqkv_hbm.at[pl.ds(r, n), pl.ds(0, 512)], wqkv_v.at[pl.ds(r, n), pl.ds(0, 512)], sem_w.at[2 + j])
            for j, (r, n) in enumerate([(0, 256), (256, 192)])]
    cp_wo = pltpu.make_async_copy(wo_hbm, wo_v, sem_w.at[4])
    cp_w1 = pltpu.make_async_copy(w1_hbm, w1_v, sem_w.at[5])
    cp_w2 = pltpu.make_async_copy(w2_hbm, w2_v, sem_w.at[6])
    cp_w3 = pltpu.make_async_copy(w3_hbm, w3_v, sem_w.at[7])
    cp_w4 = pltpu.make_async_copy(w4t_hbm, w4_v, sem_w.at[8])
    cp_x = [pltpu.make_async_copy(x_hbm.at[:, pl.ds(t * TL, TL)], x_v.at[t], sem_x.at[t]) for t in range(NT)]
    cp_o = []

    def start_out(t, r0, r1):
        cp = pltpu.make_async_copy(o_v.at[t, pl.ds(r0, r1 - r0), :],
                                   out_hbm.at[pl.ds(r0, r1 - r0), pl.ds(t * TL, TL)], sem_o.at[len(cp_o)])
        cp.start()
        cp_o.append(cp)

    def interleave(src, j, base, n):
        outs = []
        for e in range(DH // 2):
            lo = src[j, pl.ds(base + e, 8, stride=DH // 2), 0:n]
            hi = src[j, pl.ds(base + 8 * (DH // 2) + e, 8, stride=DH // 2), 0:n]
            outs.append((lo & jnp.uint32(0xFFFF)) | (hi << 16))
            outs.append((lo >> 16) | (hi & jnp.uint32(0xFFFF0000)))
        return outs

    def prep_qkv_T(ci, js=(0, 1, 2, 3)):
        c, n = QCH[ci]
        for j in js:
            r, kn = KCH[j]
            tp[j, c // 2:(c + n) // 2, 0:kn] = _pk(wqkv_v[r:r + kn, c:c + n].T)

    def prep_qkv_perm(p, js=(0, 1, 2, 3)):
        for j in js:
            r, kn = KCH[j]
            blks = interleave(tp, j, p * (D // 2), kn)
            wqkvt[p * (D // 2):(p + 1) * (D // 2), r:r + kn] = jnp.concatenate(blks, axis=0)

    def prep_wo():
        for j, (r, n) in enumerate(KCH):
            tp2[j, :, 0:n] = _pk(wo_v[:, r:r + n])
            wp = _upk(jnp.concatenate(interleave(tp2, j, 0, n), axis=0))
            wot[r // 2:(r + n) // 2, :] = _pk(wp.T)

    lane_g = lax.broadcasted_iota(jnp.int32, (DG * 8, 128), 1)

    def shifted(cur, prev, w):
        if w == 0:
            r = cur
        else:
            r = pltpu.roll(jnp.where(lane_g < 128 - DIL * w, cur, prev), DIL * w, 1)
        return _upk(r).astype(F32)

    zblk = jnp.zeros((D // 2, 128), U32)
    L1, Q, KB, VB, HB, Hs, XB, O, L2, X1, L3, U, G = ({} for _ in range(13))
    KB[-1] = zblk
    VB[-1] = zblk
    HB[-1] = zblk
    HB[NB] = zblk

    def ln1(t):
        L1[t] = _ln(x_v[t].astype(F32)).astype(BF16)

    def mm_q(t, part=None):
        if part is None:
            Q[t] = _dot(_upk(wqkvt[0:D // 2, :]), L1[t])
        elif part == 0:
            Q[t] = _dot(_upk(wqkvt[0:D // 4, :]), L1[t])
        else:
            Q[t] = jnp.concatenate([Q[t], _dot(_upk(wqkvt[D // 4:D // 2, :]), L1[t])], axis=0)

    def mm_k(t):
        kk = _pk(_dot(_upk(wqkvt[D // 2:D, :]), L1[t]).astype(BF16))
        for cb in range(NCB):
            KB[t * NCB + cb] = kk[:, cb * 128:(cb + 1) * 128]

    def mm_v(t):
        vv = _pk(_dot(_upk(wqkvt[D:3 * D // 2, :]), L1[t]).astype(BF16))
        for cb in range(NCB):
            VB[t * NCB + cb] = vv[:, cb * 128:(cb + 1) * 128]

    def attn(t):
        q = Q[t]
        cols = []
        for cb in range(NCB):
            b = t * NCB + cb
            acc = [None] * W
            for g in range(DH // DG):
                qd = q[g * DG * H:(g + 1) * DG * H, cb * 128:(cb + 1) * 128]
                cur = KB[b][g * DG * 8:(g + 1) * DG * 8, :]
                prev = KB[b - 1][g * DG * 8:(g + 1) * DG * 8, :]
                for w in range(W):
                    pr = qd * shifted(cur, prev, w)
                    s = pr[0:H]
                    for e in range(1, DG):
                        s = s + pr[e * H:(e + 1) * H]
                    acc[w] = s if acc[w] is None else acc[w] + s
            if b == 0:
                lane = lax.broadcasted_iota(jnp.int32, (H, 128), 1)
                acc = [acc[0]] + [jnp.where(lane >= DIL * w, acc[w], NEG) for w in range(1, W)]
            m = acc[0]
            for w in range(1, W):
                m = jnp.maximum(m, acc[w])
            es = [jnp.exp2((a - m) * QSCALE) for a in acc]
            den = es[0]
            for w in range(1, W):
                den = den + es[w]
            inv = 1.0 / den
            ps = [jnp.concatenate([e * inv] * DG, axis=0) for e in es]
            outs = []
            for g in range(DH // DG):
                cur = VB[b][g * DG * 8:(g + 1) * DG * 8, :]
                prev = VB[b - 1][g * DG * 8:(g + 1) * DG * 8, :]
                o = None
                for w in range(W):
                    pr = ps[w] * shifted(cur, prev, w)
                    o = pr if o is None else o + pr
                outs.append(o.astype(BF16))
            cols.append(jnp.concatenate(outs, axis=0))
        O[t] = jnp.concatenate(cols, axis=1)

    def mm_wo(t):
        h = x_v[t].astype(F32) + _dot(_upk(wot[...]), O[t])
        xb = _ln(h)
        Hs[t] = h
        XB[t] = xb
        L2[t] = _ln(xb, 0.5).astype(BF16)

    def mm_w1(t):
        hh = _pk(_gelu_half(_dot(_upk(w1t[...]), L2[t])).astype(BF16))
        for cb in range(NCB):
            HB[t * NCB + cb] = hh[:, cb * 128:(cb + 1) * 128]

    def shift(t):
        C = D // 8
        lane = lax.broadcasted_iota(jnp.int32, (C, 128), 1)
        cols = []
        for cb in range(NCB):
            b = t * NCB + cb
            cur, prv, nxt = HB[b], HB[b - 1], HB[b + 1]
            g0 = pltpu.roll(jnp.where(lane < 127, cur[0:C], prv[0:C]), 1, 1)
            g1 = pltpu.roll(jnp.where(lane >= 1, cur[C:2 * C], nxt[C:2 * C]), 127, 1)
            g2 = pltpu.roll(jnp.where(lane < 126, cur[2 * C:3 * C], prv[2 * C:3 * C]), 2, 1)
            g3 = pltpu.roll(jnp.where(lane >= 2, cur[3 * C:4 * C], nxt[3 * C:4 * C]), 126, 1)
            cols.append(jnp.concatenate([g0, g1, g2, g3], axis=0))
        G[t] = _upk(jnp.concatenate(cols, axis=1))

    def mm_w2(t):
        x1 = XB[t] + _dot(_upk(w2t[...]), G[t])
        X1[t] = Hs[t] + x1
        L3[t] = _ln(x1, 0.5).astype(BF16)

    def mm_w3(t):
        U[t] = _gelu_half(_dot(_upk(w3t[...]), L3[t])).astype(BF16)

    def mm_w4(t, r0=0, r1=D):
        o_v[t, r0:r1, :] = (X1[t][r0:r1] + _dot(w4_v[r0:r1, :], U[t])).astype(BF16)
        start_out(t, r0, r1)

    def barrier():
        pl.semaphore_signal(sem_b, 1)
        pl.semaphore_wait(sem_b, 1)

    def prep_w3(c0, c1):
        w3t[c0 // 2:c1 // 2, :] = _pk(w3_v[:, c0:c1].T)

    def mm_qkv(t):
        mm_q(t)
        mm_k(t)
        mm_v(t)

    for cp in [cp_a[0], cp_a[1], cp_x[0], cp_x[1], cp_qkv[1], cp_qkv[2], cp_x[2], cp_x[3], cp_wo, cp_x[4],
               cp_x[5], cp_w1, cp_x[6], cp_x[7], cp_w2, cp_w3, cp_w4]:
        cp.start()
        barrier()
    cp_a[0].wait()
    prep_qkv_T(0, (0, 1))
    prep_qkv_perm(0, (0, 1))
    cp_a[1].wait()
    prep_qkv_T(0, (2, 3))
    prep_qkv_perm(0, (2, 3))
    cp_x[0].wait()
    ln1(0)
    mm_q(0, 0)
    cp_x[1].wait()
    mm_q(0, 1)
    ln1(1)
    cp_qkv[1].wait()
    mm_q(1)
    prep_qkv_T(1)
    prep_qkv_perm(1)
    mm_k(0)
    cp_qkv[2].wait()
    cp_x[2].wait()
    cp_x[3].wait()
    mm_k(1)
    prep_qkv_T(2)
    prep_qkv_perm(2)
    ln1(2)
    ln1(3)
    mm_v(0)
    cp_wo.wait()
    cp_x[4].wait()
    cp_x[5].wait()
    prep_wo()
    ln1(4)
    ln1(5)
    mm_v(1)
    mm_qkv(2)
    mm_qkv(3)
    attn(0)
    attn(1)
    cp_w1.wait()
    cp_x[6].wait()
    cp_x[7].wait()
    cp_w2.wait()
    w1t[...] = _pk(w1_v[...].T)
    w2t[...] = _pk(w2_v[...].T)
    ln1(6)
    ln1(7)
    mm_wo(0)
    mm_wo(1)
    mm_qkv(4)
    mm_q(5)
    mm_k(5)
    mm_w1(0)
    mm_w1(1)
    mm_v(5)
    attn(2)
    attn(3)
    shift(0)
    cp_w3.wait()
    prep_w3(0, F)
    mm_wo(2)
    mm_wo(3)
    mm_w2(0)
    mm_qkv(6)
    mm_q(7)
    mm_k(7)
    mm_w1(2)
    mm_w1(3)
    mm_v(7)
    attn(4)
    attn(5)
    shift(1)
    shift(2)
    cp_w4.wait()
    mm_wo(4)
    mm_wo(5)
    mm_w2(1)
    mm_w2(2)
    mm_w3(0)
    mm_w1(4)
    mm_w1(5)
    mm_w4(0)
    attn(6)
    attn(7)
    shift(3)
    shift(4)
    barrier()
    mm_wo(6)
    mm_wo(7)
    mm_w2(3)
    mm_w2(4)
    mm_w3(1)
    mm_w1(6)
    mm_w1(7)
    mm_w4(1)
    shift(5)
    shift(6)
    shift(7)
    mm_w3(2)
    mm_w2(5)
    mm_w2(6)
    mm_w2(7)
    mm_w4(2)
    for t in range(3, 7):
        mm_w3(t)
        if t > 3:
            mm_w4(t - 1)
    mm_w3(7)
    mm_w4(6)
    mm_w4(7, 0, 320)
    mm_w4(7, 320, D)
    for cp in cp_o:
        cp.wait()


@jax.jit
def pallas_sequential_preLN__sliding_local_dilated__mixer_s_mlp__prompt_kernel(
    A_x, A_wqkv, A_wo, B_x, B_w1, B_w2, B_w3, B_w4,
):
    xt = A_x.reshape(S, D).T
    w4t = B_w4.T
    anyspec = pl.BlockSpec(memory_space=pl.ANY)
    out = pl.pallas_call(
        _kernel,
        in_specs=[anyspec] * 7,
        out_specs=anyspec,
        out_shape=jax.ShapeDtypeStruct((D, S), BF16),
        scratch_shapes=[
            pltpu.VMEM((NT, D, TL), BF16),
            pltpu.VMEM((NT, D, TL), BF16),
            pltpu.VMEM((D, 3 * D), BF16),
            pltpu.VMEM((D, D), BF16),
            pltpu.VMEM((D, D), BF16),
            pltpu.VMEM((D, D), BF16),
            pltpu.VMEM((D, F), BF16),
            pltpu.VMEM((D, F), BF16),
            pltpu.VMEM((3 * D // 2, D), U32),
            pltpu.VMEM((D // 2, D), U32),
            pltpu.VMEM((D // 2, D), U32),
            pltpu.VMEM((D // 2, D), U32),
            pltpu.VMEM((F // 2, D), U32),
            pltpu.VMEM((4, 3 * D // 2, 128), U32),
            pltpu.VMEM((4, D // 2, 128), U32),
            pltpu.SemaphoreType.DMA((9,)),
            pltpu.SemaphoreType.DMA((NT,)),
            pltpu.SemaphoreType.DMA((NT + 1,)),
            pltpu.SemaphoreType.REGULAR,
        ],
        compiler_params=pltpu.CompilerParams(vmem_limit_bytes=100 * 1024 * 1024),
    )(xt, A_wqkv, A_wo, B_w1, B_w2, B_w3, w4t)
    return out.T.reshape(1, S, D)
```

```python
import jax
import jax.numpy as jnp
from jax import lax
import jax.experimental.pallas as pl
import jax.experimental.pallas.tpu as pltpu

S, D, H, DH, W, DIL, F = 2048, 448, 16, 28, 8, 2, 1792
TL = 256
NT = S // TL
NCB = TL // 128
NB = S // 128
EPS = 1e-5
LOG2E = 1.4426950408889634
QSCALE = (DH ** -0.5) * LOG2E
NEG = -1e9 * (DH ** 0.5)
WORD = (1, 2, 3, 4, 5, 6, 7, 0)
F32, BF16, U32 = jnp.float32, jnp.bfloat16, jnp.uint32
KCH = [(0, 128), (128, 128), (256, 128), (384, 64)]
QCH = [(0, 512), (512, 384), (896, 448)]
W4CH = 224
LAST = 128


def _colmean(x):
    return jnp.sum(x, axis=0, keepdims=True) * (1.0 / D)


def _affine(x, m, r):
    return x * r - m * r


def _gelu_half(hx):
    c0 = 2.0 * 0.7978845608028654
    c1 = 8.0 * 0.7978845608028654 * 0.044715
    t = jnp.tanh(hx * (c0 + c1 * (hx * hx)))
    return hx + hx * t


def _dot(a, b):
    return jnp.dot(a, b, preferred_element_type=F32)


def _pk(x_bf16):
    return pltpu.bitcast(x_bf16, U32)


def _upk(x_u32):
    return pltpu.bitcast(x_u32, BF16)


def _pack16(x):
    n = x.shape[0] // 16
    x4 = x.reshape(n, 2, 8, x.shape[1])
    p = pltpu.pack_elementwise([x4[:, 0], x4[:, 1]], packed_dtype=BF16)
    return p.reshape(n * 8, x.shape[1])


def _unpack16(p):
    lo = pltpu.unpack_elementwise(p, index=0, packed_dtype=BF16, unpacked_dtype=F32)
    hi = pltpu.unpack_elementwise(p, index=1, packed_dtype=BF16, unpacked_dtype=F32)
    return jnp.concatenate([lo, hi], axis=0)


def _kernel(x_hbm, wqkv_hbm, wo_hbm, w1_hbm, w2_hbm, w3_hbm, w4t_hbm, out_hbm,
            x_v, o_v, o_last, wa1_v, wa2_v, wb_v, wc_v, wo_v, w1_v, w2_v, w3_v, w4_v,
            wqkvt, wot, w1t, w2t, w3t, tp, tp2, q_s, w4t, o_s,
            sem_w, sem_x, sem_o, sem_b):
    cp_qkv = [None,
              pltpu.make_async_copy(wqkv_hbm.at[:, pl.ds(*QCH[1])], wb_v, sem_w.at[0]),
              pltpu.make_async_copy(wqkv_hbm.at[:, pl.ds(*QCH[2])], wc_v, sem_w.at[1])]
    cp_a = [pltpu.make_async_copy(wqkv_hbm.at[pl.ds(0, 256), pl.ds(*QCH[0])], wa1_v, sem_w.at[2]),
            pltpu.make_async_copy(wqkv_hbm.at[pl.ds(256, D - 256), pl.ds(*QCH[0])], wa2_v, sem_w.at[3])]
    cp_wo = pltpu.make_async_copy(wo_hbm, wo_v, sem_w.at[4])
    cp_w1 = pltpu.make_async_copy(w1_hbm, w1_v, sem_w.at[5])
    cp_w2 = pltpu.make_async_copy(w2_hbm, w2_v, sem_w.at[6])
    cp_w3 = pltpu.make_async_copy(w3_hbm, w3_v, sem_w.at[7])
    cp_w4 = pltpu.make_async_copy(w4t_hbm, w4_v, sem_w.at[8])
    cp_x = [pltpu.make_async_copy(x_hbm.at[:, pl.ds(t * TL, TL)], x_v.at[t], sem_x.at[t]) for t in range(NT)]
    cp_o = []

    def start_out(src, t, r0, r1):
        cp = pltpu.make_async_copy(src, out_hbm.at[pl.ds(r0, r1 - r0), pl.ds(t * TL, TL)], sem_o.at[len(cp_o)])
        cp.start()
        cp_o.append(cp)

    def interleave(src, j, base, n, adjacent):
        outs = []
        for e in range(DH // 2):
            if adjacent:
                lo = src[j, pl.ds(base + e, 8, stride=DH), 0:n]
                hi = src[j, pl.ds(base + DH // 2 + e, 8, stride=DH), 0:n]
            else:
                lo = src[j, pl.ds(base + e, 8, stride=DH // 2), 0:n]
                hi = src[j, pl.ds(base + 8 * (DH // 2) + e, 8, stride=DH // 2), 0:n]
            outs.append((lo & jnp.uint32(0xFFFF)) | (hi << 16))
            outs.append((lo >> 16) | (hi & jnp.uint32(0xFFFF0000)))
        return outs

    def prep_qkv_T(ci, js=(0, 1, 2, 3)):
        c, n = QCH[ci]
        for j in js:
            r, kn = KCH[j]
            if ci == 0:
                blk = wa1_v[r:r + kn, :] if r < 256 else wa2_v[r - 256:r - 256 + kn, :]
            else:
                blk = (wb_v, wc_v)[ci - 1][r:r + kn, :]
            tp[j, c // 2:(c + n) // 2, 0:kn] = _pk(blk.T)

    def prep_qkv_perm(p, js=(0, 1, 2, 3)):
        for j in js:
            r, kn = KCH[j]
            blks = interleave(tp, j, p * (D // 2), kn, True)
            wqkvt[p * (D // 2):(p + 1) * (D // 2), r:r + kn] = jnp.concatenate(blks, axis=0)

    def prep_wo():
        for j, (r, n) in enumerate(KCH):
            tp2[j, :, 0:n] = _pk(wo_v[:, r:r + n])
            wp = _upk(jnp.concatenate(interleave(tp2, j, 0, n, False), axis=0))
            wot[r // 2:(r + n) // 2, :] = _pk(wp.T)

    lane8 = lax.broadcasted_iota(jnp.int32, (8, 128), 1)

    def shifted(cur, prev, w):
        if w == 0:
            r = cur
        else:
            r = pltpu.roll(jnp.where(lane8 < 128 - DIL * w, cur, prev), DIL * w, 1)
        return _unpack16(r)

    zblk = jnp.zeros((D // 2, 128), U32)
    L1, Q, KB, VB, HB, Hs, XB, L2, X1, L3, U, G = ({} for _ in range(12))
    KB[-1] = zblk
    VB[-1] = zblk
    HB[-1] = zblk
    HB[NB] = zblk

    def ln1(t):
        x = x_v[t].astype(F32)
        xc = x - _colmean(x)
        L1[t] = (xc * lax.rsqrt(_colmean(xc * xc) + EPS)).astype(BF16)

    def mm_q(t, part=None):
        if part is None:
            Q[t] = _dot(_upk(wqkvt[0:D // 2, :]), L1[t])
        elif part == 0:
            q_s[...] = _dot(_upk(wqkvt[0:D // 2, 0:256]), L1[t][0:256])
        else:
            Q[t] = q_s[...] + _dot(_upk(wqkvt[0:D // 2, 256:D]), L1[t][256:D])

    def mm_k(t):
        kk = _pack16(_dot(_upk(wqkvt[D // 2:D, :]), L1[t]))
        for cb in range(NCB):
            KB[t * NCB + cb] = kk[:, cb * 128:(cb + 1) * 128]

    def mm_v(t):
        vv = _pack16(_dot(_upk(wqkvt[D:3 * D // 2, :]), L1[t]))
        for cb in range(NCB):
            VB[t * NCB + cb] = vv[:, cb * 128:(cb + 1) * 128]

    def probs(b):
        t, cb = divmod(b, NCB)
        acc = [None] * W
        for w in WORD:
            for g in range(DH):
                qd = Q[t][g * H:(g + 1) * H, cb * 128:(cb + 1) * 128]
                s = qd * shifted(KB[b][g * 8:(g + 1) * 8, :], KB[b - 1][g * 8:(g + 1) * 8, :], w)
                acc[w] = s if acc[w] is None else acc[w] + s
        if b == 0:
            lane = lax.broadcasted_iota(jnp.int32, (H, 128), 1)
            acc = [acc[0]] + [jnp.where(lane >= DIL * w, acc[w], NEG) for w in range(1, W)]
        m = acc[0]
        for w in range(1, W):
            m = jnp.maximum(m, acc[w])
        es = [jnp.exp2((a - m) * QSCALE) for a in acc]
        den = es[0]
        for w in range(1, W):
            den = den + es[w]
        inv = 1.0 / den
        return [e * inv for e in es]

    def pv(b, ps):
        outs = [None] * DH
        for g in range(DH):
            for w in WORD:
                pr = ps[w] * shifted(VB[b][g * 8:(g + 1) * 8, :], VB[b - 1][g * 8:(g + 1) * 8, :], w)
                outs[g] = pr if outs[g] is None else outs[g] + pr
        return jnp.concatenate([_pack16(o) for o in outs], axis=0)

    def attn(t):
        bs = [t * NCB + cb for cb in range(NCB)]
        o_s[t] = jnp.concatenate([pv(b, probs(b)) for b in bs], axis=1)

    def mm_wo(t):
        h = x_v[t].astype(F32) + _dot(_upk(wot[...]), _upk(o_s[t]))
        m = _colmean(h)
        hc = h - m
        v = _colmean(hc * hc)
        r = lax.rsqrt(v + EPS)
        Hs[t] = h
        XB[t] = (m, r)
        m2 = r * _colmean(hc)
        v2 = jnp.maximum(r * r * v - m2 * m2, 0.0)
        r2 = lax.rsqrt(v2 + EPS) * 0.5
        L2[t] = (h * (r * r2) - (m * r + m2) * r2).astype(BF16)

    def mm_w1(t):
        hh = _pack16(_gelu_half(_dot(_upk(w1t[...]), L2[t])))
        for cb in range(NCB):
            HB[t * NCB + cb] = hh[:, cb * 128:(cb + 1) * 128]

    def shift(t):
        C = D // 8
        lane = lax.broadcasted_iota(jnp.int32, (C, 128), 1)
        cols = []
        for cb in range(NCB):
            b = t * NCB + cb
            cur, prv, nxt = HB[b], HB[b - 1], HB[b + 1]
            g0 = pltpu.roll(jnp.where(lane < 127, cur[0:C], prv[0:C]), 1, 1)
            g1 = pltpu.roll(jnp.where(lane >= 1, cur[C:2 * C], nxt[C:2 * C]), 127, 1)
            g2 = pltpu.roll(jnp.where(lane < 126, cur[2 * C:3 * C], prv[2 * C:3 * C]), 2, 1)
            g3 = pltpu.roll(jnp.where(lane >= 2, cur[3 * C:4 * C], nxt[3 * C:4 * C]), 126, 1)
            cols.append(jnp.concatenate([g0, g1, g2, g3], axis=0))
        G[t] = _upk(jnp.concatenate(cols, axis=1))

    def mm_w2(t):
        x1 = _affine(Hs[t], *XB[t]) + _dot(_upk(w2t[...]), G[t])
        X1[t] = x1
        m = _colmean(x1)
        xc = x1 - m
        r = lax.rsqrt(_colmean(xc * xc) + EPS) * 0.5
        L3[t] = _affine(x1, m, r).astype(BF16)

    def mm_w3(t):
        U[t] = _gelu_half(_dot(_upk(w3t[...]), L3[t])).astype(BF16)

    def mm_w4(t, r0=0, r1=D):
        for c0 in range(r0, r1, W4CH):
            c1 = min(c0 + W4CH, r1)
            res = (Hs[t][c0:c1] + X1[t][c0:c1] + _dot(_upk(w4t[c0 // 2:c1 // 2, :]), U[t])).astype(BF16)
            if r0 == 0:
                o_v[t, c0:c1, :] = res
            else:
                o_last[c0 - r0:c1 - r0, :] = res
        start_out(o_v.at[t, pl.ds(0, r1), :] if r0 == 0 else o_last, t, r0, r1)

    def barrier():
        pl.semaphore_signal(sem_b, 1)
        pl.semaphore_wait(sem_b, 1)

    def mm_qkv(t):
        mm_q(t)
        mm_k(t)
        mm_v(t)

    for cp in [cp_x[0], cp_a[0], cp_a[1], cp_x[1], cp_x[2], cp_qkv[1], cp_x[3], cp_qkv[2], cp_x[4], cp_wo,
               cp_x[5], cp_x[6], cp_w1, cp_x[7], cp_w2, cp_w3, cp_w4]:
        cp.start()
        barrier()
    cp_x[0].wait()
    ln1(0)
    cp_a[0].wait()
    prep_qkv_T(0, (0, 1))
    prep_qkv_perm(0, (0, 1))
    cp_a[1].wait()
    mm_q(0, 0)
    prep_qkv_T(0, (2, 3))
    prep_qkv_perm(0, (2, 3))
    cp_x[1].wait()
    mm_q(0, 1)
    ln1(1)
    cp_x[2].wait()
    mm_q(1)
    ln1(2)
    cp_qkv[1].wait()
    mm_q(2)
    prep_qkv_T(1)
    prep_qkv_perm(1)
    mm_k(0)
    mm_k(1)
    cp_x[3].wait()
    cp_qkv[2].wait()
    cp_x[4].wait()
    mm_k(2)
    prep_qkv_T(2)
    prep_qkv_perm(2)
    ln1(3)
    ln1(4)
    mm_v(0)
    cp_wo.wait()
    cp_x[5].wait()
    cp_x[6].wait()
    prep_wo()
    ln1(5)
    ln1(6)
    mm_v(1)
    mm_v(2)
    mm_qkv(3)
    mm_q(4)
    mm_k(4)
    attn(0)
    attn(1)
    cp_w1.wait()
    cp_x[7].wait()
    cp_w2.wait()
    w1t[...] = _pk(w1_v[...].T)
    w2t[...] = _pk(_upk(_pack16(w2_v[...].astype(F32))).T)
    ln1(7)
    mm_wo(0)
    mm_wo(1)
    mm_v(4)
    mm_qkv(5)
    mm_q(6)
    mm_w1(0)
    mm_w1(1)
    mm_k(6)
    attn(2)
    attn(3)
    shift(0)
    cp_w3.wait()
    w3t[...] = _pk(w3_v[...].T)
    mm_wo(2)
    mm_wo(3)
    mm_w2(0)
    mm_v(6)
    mm_q(7)
    mm_k(7)
    mm_w1(2)
    mm_w1(3)
    mm_v(7)
    attn(4)
    attn(5)
    cp_w4.wait()
    w4t[...] = _pk(w4_v[...])
    shift(1)
    shift(2)
    mm_wo(4)
    mm_w2(1)
    mm_wo(5)
    mm_w2(2)
    mm_w3(0)
    mm_w1(4)
    mm_w1(5)
    mm_w4(0)
    attn(6)
    attn(7)
    barrier()
    shift(3)
    shift(4)
    mm_wo(6)
    mm_wo(7)
    mm_w2(3)
    mm_w2(4)
    mm_w3(1)
    mm_w1(6)
    mm_w1(7)
    mm_w4(1)
    shift(5)
    shift(6)
    shift(7)
    mm_w3(2)
    mm_w2(5)
    mm_w2(6)
    mm_w2(7)
    mm_w4(2)
    for t in range(3, 7):
        mm_w3(t)
        if t > 3:
            mm_w4(t - 1)
    mm_w3(7)
    mm_w4(6)
    mm_w4(7, 0, D - LAST)
    mm_w4(7, D - LAST, D)
    for cp in cp_o:
        cp.wait()


@jax.jit
def pallas_sequential_preLN__sliding_local_dilated__mixer_s_mlp__prompt_kernel(
    A_x, A_wqkv, A_wo, B_x, B_w1, B_w2, B_w3, B_w4,
):
    xt = A_x.reshape(S, D).T
    w4t = B_w4.T
    anyspec = pl.BlockSpec(memory_space=pl.ANY)
    out = pl.pallas_call(
        _kernel,
        in_specs=[anyspec] * 7,
        out_specs=anyspec,
        out_shape=jax.ShapeDtypeStruct((D, S), BF16),
        scratch_shapes=[
            pltpu.VMEM((NT, D, TL), BF16),
            pltpu.VMEM((NT, D, TL), BF16),
            pltpu.VMEM((LAST, TL), BF16),
            pltpu.VMEM((256, 512), BF16),
            pltpu.VMEM((D - 256, 512), BF16),
            pltpu.VMEM((D, 384), BF16),
            pltpu.VMEM((D, D), BF16),
            pltpu.VMEM((D, D), BF16),
            pltpu.VMEM((D, D), BF16),
            pltpu.VMEM((D, D), BF16),
            pltpu.VMEM((D, F), BF16),
            pltpu.VMEM((D, F), BF16),
            pltpu.VMEM((3 * D // 2, D), U32),
            pltpu.VMEM((D // 2, D), U32),
            pltpu.VMEM((D // 2, D), U32),
            pltpu.VMEM((D // 2, D), U32),
            pltpu.VMEM((F // 2, D), U32),
            pltpu.VMEM((4, 3 * D // 2, 128), U32),
            pltpu.VMEM((4, D // 2, 128), U32),
            pltpu.VMEM((D, TL), F32),
            pltpu.VMEM((D // 2, F), U32),
            pltpu.VMEM((NT, D // 2, TL), U32),
            pltpu.SemaphoreType.DMA((9,)),
            pltpu.SemaphoreType.DMA((NT,)),
            pltpu.SemaphoreType.DMA((NT + 1,)),
            pltpu.SemaphoreType.REGULAR,
        ],
        compiler_params=pltpu.CompilerParams(vmem_limit_bytes=100 * 1024 * 1024),
    )(xt, A_wqkv, A_wo, B_w1, B_w2, B_w3, w4t)
    return out.T.reshape(1, S, D)
```

```python
import jax
import jax.numpy as jnp
from jax import lax
import jax.experimental.pallas as pl
import jax.experimental.pallas.tpu as pltpu

S, D, H, DH, W, DIL, F = 2048, 448, 16, 28, 8, 2, 1792
TL = 256
NT = S // TL
NCB = TL // 128
NB = S // 128
EPS = 1e-5
LOG2E = 1.4426950408889634
QSCALE = (DH ** -0.5) * LOG2E
NEG = -1e9 * (DH ** 0.5)
WORD = (0, 1, 2, 3, 4, 5, 6, 7)
F32, BF16, U32 = jnp.float32, jnp.bfloat16, jnp.uint32
KCH = [(0, 128), (128, 128), (256, 128), (384, 64)]
QCH = [(0, 512), (512, 384), (896, 448)]
W4CH = 224
LAST = 64


def _colmean(x):
    return jnp.sum(x, axis=0, keepdims=True) * (1.0 / D)


def _affine(x, m, r):
    return x * r - m * r


GA = 0.7978845608028654
GBETA = (GA * 0.044715) ** (1.0 / 3.0)
GOUT = 0.5 / GBETA


def _gelu_scaled(y):
    t = jnp.tanh(y * (GA / GBETA + y * y))
    return y + y * t


def _dot(a, b):
    return jnp.dot(a, b, preferred_element_type=F32)


def _pk(x_bf16):
    return pltpu.bitcast(x_bf16, U32)


def _upk(x_u32):
    return pltpu.bitcast(x_u32, BF16)


def _unpack16(p):
    lo = lax.bitcast_convert_type(p << 16, F32)
    hi = lax.bitcast_convert_type(p & jnp.uint32(0xFFFF0000), F32)
    return jnp.concatenate([lo, hi], axis=0)


def _kernel(x_hbm, wqkv_hbm, wo_hbm, w1_hbm, w2_hbm, w3_hbm, w4t_hbm, out_hbm,
            x_v, o_v, o_last, wa1_v, wa2_v, wb_v, wc_v, wo_v, w1_v, w2_v, w3_v, w4_v,
            wqkvt, wot, w1t, w2t, w3t, tp, tp2, q_s, w4t,
            sem_w, sem_x, sem_o, sem_b):
    cp_qkv = [None,
              pltpu.make_async_copy(wqkv_hbm.at[:, pl.ds(*QCH[1])], wb_v, sem_w.at[0]),
              pltpu.make_async_copy(wqkv_hbm.at[:, pl.ds(*QCH[2])], wc_v, sem_w.at[1])]
    cp_a = [pltpu.make_async_copy(wqkv_hbm.at[pl.ds(0, 256), pl.ds(*QCH[0])], wa1_v, sem_w.at[2]),
            pltpu.make_async_copy(wqkv_hbm.at[pl.ds(256, D - 256), pl.ds(*QCH[0])], wa2_v, sem_w.at[3])]
    cp_wo = pltpu.make_async_copy(wo_hbm, wo_v, sem_w.at[4])
    cp_w1 = pltpu.make_async_copy(w1_hbm, w1_v, sem_w.at[5])
    cp_w2 = pltpu.make_async_copy(w2_hbm, w2_v, sem_w.at[6])
    cp_w3 = pltpu.make_async_copy(w3_hbm, w3_v, sem_w.at[7])
    cp_w4 = pltpu.make_async_copy(w4t_hbm, w4_v, sem_w.at[8])
    cp_x = [pltpu.make_async_copy(x_hbm.at[:, pl.ds(t * TL, TL)], x_v.at[t], sem_x.at[t]) for t in range(NT)]
    cp_o = []

    def start_out(src, t, r0, r1):
        cp = pltpu.make_async_copy(src, out_hbm.at[pl.ds(r0, r1 - r0), pl.ds(t * TL, TL)], sem_o.at[len(cp_o)])
        cp.start()
        cp_o.append(cp)

    def interleave(src, j, base, n, adjacent):
        outs = []
        for e in range(DH // 2):
            if adjacent:
                lo = src[j, pl.ds(base + e, 8, stride=DH), 0:n]
                hi = src[j, pl.ds(base + DH // 2 + e, 8, stride=DH), 0:n]
            else:
                lo = src[j, pl.ds(base + e, 8, stride=DH // 2), 0:n]
                hi = src[j, pl.ds(base + 8 * (DH // 2) + e, 8, stride=DH // 2), 0:n]
            outs.append((lo & jnp.uint32(0xFFFF)) | (hi << 16))
            outs.append((lo >> 16) | (hi & jnp.uint32(0xFFFF0000)))
        return outs

    def prep_qkv_T(ci, js=(0, 1, 2, 3)):
        c, n = QCH[ci]
        for j in js:
            r, kn = KCH[j]
            if ci == 0:
                blk = wa1_v[r:r + kn, :] if r < 256 else wa2_v[r - 256:r - 256 + kn, :]
            else:
                blk = (wb_v, wc_v)[ci - 1][r:r + kn, :]
            tp[j, c // 2:(c + n) // 2, 0:kn] = _pk(blk.T)

    def prep_qkv_perm(p, js=(0, 1, 2, 3)):
        for j in js:
            r, kn = KCH[j]
            blks = interleave(tp, j, p * (D // 2), kn, p == 0)
            wqkvt[p * (D // 2):(p + 1) * (D // 2), r:r + kn] = jnp.concatenate(blks, axis=0)

    def prep_wo():
        for j, (r, n) in enumerate(KCH):
            tp2[j, 0:D // 2, 0:n] = _pk(wo_v[:, r:r + n])
            wp = _upk(jnp.concatenate(interleave(tp2, j, 0, n, True), axis=0))
            wot[r // 2:(r + n) // 2, :] = _pk(wp.T)

    lane8 = lax.broadcasted_iota(jnp.int32, (8, 128), 1)

    def shifted(cur, prev, w):
        if w == 0:
            r = cur
        else:
            r = pltpu.roll(jnp.where(lane8 < 128 - DIL * w, cur, prev), DIL * w, 1)
        return _unpack16(r)

    zblk = jnp.zeros((D // 2, 128), U32)
    L1, Q, KB, VB, HB, Hs, XB, L2, X1, L3, U, G, O = ({} for _ in range(13))
    KB[-1] = zblk
    VB[-1] = zblk
    HB[-1] = jnp.zeros((D, 128), F32)
    HB[NB] = jnp.zeros((D, 128), F32)

    def ln1(t):
        x = x_v[t].astype(F32)
        xc = x - _colmean(x)
        L1[t] = (xc * lax.rsqrt(_colmean(xc * xc) + EPS)).astype(BF16)

    def mm_q(t, part=None):
        if part is None:
            Q[t] = _dot(_upk(wqkvt[0:D // 2, :]), L1[t])
        elif part == 0:
            q_s[...] = _dot(_upk(wqkvt[0:D // 2, 0:256]), L1[t][0:256])
        else:
            Q[t] = q_s[...] + _dot(_upk(wqkvt[0:D // 2, 256:D]), L1[t][256:D])

    def mm_k(t):
        kk = _pk(_dot(_upk(wqkvt[D // 2:D, :]), L1[t]).astype(BF16))
        for cb in range(NCB):
            KB[t * NCB + cb] = kk[:, cb * 128:(cb + 1) * 128]

    def mm_v(t):
        vv = _pk(_dot(_upk(wqkvt[D:3 * D // 2, :]), L1[t]).astype(BF16))
        for cb in range(NCB):
            VB[t * NCB + cb] = vv[:, cb * 128:(cb + 1) * 128]

    def probs(b):
        t, cb = divmod(b, NCB)
        acc = [None] * W
        for w in WORD:
            for g in range(DH):
                qd = Q[t][g * H:(g + 1) * H, cb * 128:(cb + 1) * 128]
                s = qd * shifted(KB[b][g * 8:(g + 1) * 8, :], KB[b - 1][g * 8:(g + 1) * 8, :], w)
                acc[w] = s if acc[w] is None else acc[w] + s
        if b == 0:
            lane = lax.broadcasted_iota(jnp.int32, (H, 128), 1)
            acc = [acc[0]] + [jnp.where(lane >= DIL * w, acc[w], NEG) for w in range(1, W)]
        m = acc[0]
        for w in range(1, W):
            m = jnp.maximum(m, acc[w])
        es = [jnp.exp2((a - m) * QSCALE) for a in acc]
        den = es[0]
        for w in range(1, W):
            den = den + es[w]
        r0 = pl.reciprocal(den, approx=True)
        inv = r0 * (2.0 - den * r0)
        return [e * inv for e in es]

    def pv(b, ps):
        outs = [None] * DH
        for g in range(DH):
            for w in WORD:
                pr = ps[w] * shifted(VB[b][g * 8:(g + 1) * 8, :], VB[b - 1][g * 8:(g + 1) * 8, :], w)
                outs[g] = pr if outs[g] is None else outs[g] + pr
        return jnp.concatenate(outs, axis=0)

    def attn(t):
        bs = [t * NCB + cb for cb in range(NCB)]
        O[t] = jnp.concatenate([pv(b, probs(b)) for b in bs], axis=1).astype(BF16)

    def mm_wo(t):
        h = x_v[t].astype(F32) + _dot(_upk(wot[...]), O[t])
        m = _colmean(h)
        hc = h - m
        v = _colmean(hc * hc)
        r = lax.rsqrt(v + EPS)
        Hs[t] = h
        XB[t] = (m, r)
        m2 = r * _colmean(hc)
        v2 = jnp.maximum(r * r * v - m2 * m2, 0.0)
        r2 = lax.rsqrt(v2 + EPS) * GBETA
        L2[t] = (h * (r * r2) - (m * r + m2) * r2).astype(BF16)

    def mm_w1(t):
        hh = _gelu_scaled(_dot(_upk(w1t[...]), L2[t]))
        for cb in range(NCB):
            HB[t * NCB + cb] = hh[:, cb * 128:(cb + 1) * 128]

    def shift(t):
        C = D // 4
        lane = lax.broadcasted_iota(jnp.int32, (C, 128), 1)
        cols = []
        for cb in range(NCB):
            b = t * NCB + cb
            cur, prv, nxt = HB[b], HB[b - 1], HB[b + 1]
            g0 = pltpu.roll(jnp.where(lane < 127, cur[0:C], prv[0:C]), 1, 1)
            g1 = pltpu.roll(jnp.where(lane >= 1, cur[C:2 * C], nxt[C:2 * C]), 127, 1)
            g2 = pltpu.roll(jnp.where(lane < 126, cur[2 * C:3 * C], prv[2 * C:3 * C]), 2, 1)
            g3 = pltpu.roll(jnp.where(lane >= 2, cur[3 * C:4 * C], nxt[3 * C:4 * C]), 126, 1)
            cols.append(jnp.concatenate([g0, g1, g2, g3], axis=0))
        G[t] = jnp.concatenate(cols, axis=1).astype(BF16)

    def mm_w2(t):
        m0, r0 = XB[t]
        x1s = _affine(Hs[t], m0, r0 * (1.0 / GOUT)) + _dot(_upk(w2t[...]), G[t])
        X1[t] = x1s
        m = _colmean(x1s)
        xc = x1s - m
        r = lax.rsqrt(_colmean(xc * xc) + EPS / (GOUT * GOUT)) * GBETA
        L3[t] = _affine(x1s, m, r).astype(BF16)

    def mm_w3(t):
        U[t] = _gelu_scaled(_dot(_upk(w3t[...]), L3[t])).astype(BF16)

    def w4_rows(t, c0, c1):
        return (Hs[t][c0:c1] + GOUT * (X1[t][c0:c1] + _dot(_upk(w4t[c0 // 2:c1 // 2, :]), U[t]))).astype(BF16)

    def mm_w4a(t):
        o_v[t, 0:W4CH, :] = w4_rows(t, 0, W4CH)

    def mm_w4b(t, r1=D):
        o_v[t, W4CH:r1, :] = w4_rows(t, W4CH, r1)
        start_out(o_v.at[t, pl.ds(0, r1), :], t, 0, r1)

    def mm_w4(t):
        mm_w4a(t)
        mm_w4b(t)

    def barrier():
        pl.semaphore_signal(sem_b, 1)
        pl.semaphore_wait(sem_b, 1)

    def mm_qkv(t):
        mm_q(t)
        mm_k(t)
        mm_v(t)

    for cp in [cp_x[0], cp_a[0], cp_a[1], cp_x[1], cp_x[2], cp_qkv[1], cp_x[3], cp_qkv[2], cp_x[4], cp_x[5],
               cp_x[6], cp_wo, cp_x[7], cp_w1, cp_w2, cp_w3, cp_w4]:
        cp.start()
        barrier()
    cp_x[0].wait()
    ln1(0)
    cp_a[0].wait()
    prep_qkv_T(0, (0, 1))
    prep_qkv_perm(0, (0, 1))
    cp_a[1].wait()
    mm_q(0, 0)
    prep_qkv_T(0, (2, 3))
    prep_qkv_perm(0, (2, 3))
    cp_x[1].wait()
    mm_q(0, 1)
    ln1(1)
    cp_x[2].wait()
    mm_q(1)
    ln1(2)
    cp_qkv[1].wait()
    mm_q(2)
    prep_qkv_T(1)
    prep_qkv_perm(1)
    mm_k(0)
    mm_k(1)
    cp_x[3].wait()
    cp_qkv[2].wait()
    cp_x[4].wait()
    cp_x[5].wait()
    mm_k(2)
    prep_qkv_T(2)
    prep_qkv_perm(2)
    ln1(3)
    ln1(4)
    ln1(5)
    mm_v(0)
    mm_v(1)
    cp_wo.wait()
    cp_x[6].wait()
    ln1(6)
    prep_wo()
    mm_v(2)
    mm_qkv(3)
    mm_qkv(4)
    attn(0)
    attn(1)
    cp_w1.wait()
    cp_x[7].wait()
    w1t[...] = _pk(w1_v[...].T)
    ln1(7)
    mm_wo(0)
    mm_wo(1)
    mm_qkv(5)
    mm_q(6)
    mm_w1(0)
    mm_w1(1)
    mm_k(6)
    attn(2)
    attn(3)
    cp_w2.wait()
    cp_w3.wait()
    w3t[...] = _pk(w3_v[...].T)
    shift(0)
    w2t[...] = _pk(w2_v[...].T)
    mm_wo(2)
    mm_wo(3)
    mm_v(6)
    mm_q(7)
    mm_w2(0)
    mm_k(7)
    mm_w1(2)
    mm_w1(3)
    mm_w3(0)
    mm_v(7)
    attn(4)
    attn(5)
    cp_w4.wait()
    shift(1)
    w4t[...] = _pk(w4_v[...])
    mm_wo(4)
    mm_wo(5)
    mm_w2(1)
    mm_w4a(0)
    mm_w1(4)
    mm_w1(5)
    mm_w3(1)
    mm_w4b(0)
    attn(6)
    attn(7)
    barrier()
    shift(2)
    shift(3)
    shift(4)
    mm_wo(6)
    mm_wo(7)
    mm_w2(2)
    mm_w2(3)
    mm_w2(4)
    mm_w1(6)
    mm_w4(1)
    mm_w1(7)
    shift(5)
    shift(6)
    shift(7)
    mm_w3(2)
    mm_w2(5)
    mm_w3(3)
    mm_w2(6)
    mm_w3(4)
    mm_w2(7)
    mm_w4(2)
    mm_w4(3)
    mm_w4(4)
    mm_w3(5)
    mm_w3(6)
    mm_w3(7)
    mm_w4(5)
    mm_w4(6)
    mm_w4a(7)
    mm_w4b(7, D - LAST)
    o_last[...] = w4_rows(7, D - LAST, D)
    start_out(o_last, 7, D - LAST, D)
    for cp in cp_o:
        cp.wait()


@jax.jit
def pallas_sequential_preLN__sliding_local_dilated__mixer_s_mlp__prompt_kernel(
    A_x, A_wqkv, A_wo, B_x, B_w1, B_w2, B_w3, B_w4,
):
    xt = A_x.reshape(S, D).T
    w4t = B_w4.T
    anyspec = pl.BlockSpec(memory_space=pl.ANY)
    out = pl.pallas_call(
        _kernel,
        in_specs=[anyspec] * 7,
        out_specs=anyspec,
        out_shape=jax.ShapeDtypeStruct((D, S), BF16),
        scratch_shapes=[
            pltpu.VMEM((NT, D, TL), BF16),
            pltpu.VMEM((NT, D, TL), BF16),
            pltpu.VMEM((LAST, TL), BF16),
            pltpu.VMEM((256, 512), BF16),
            pltpu.VMEM((D - 256, 512), BF16),
            pltpu.VMEM((D, 384), BF16),
            pltpu.VMEM((D, D), BF16),
            pltpu.VMEM((D, D), BF16),
            pltpu.VMEM((D, D), BF16),
            pltpu.VMEM((D, D), BF16),
            pltpu.VMEM((D, F), BF16),
            pltpu.VMEM((D, F), BF16),
            pltpu.VMEM((3 * D // 2, D), U32),
            pltpu.VMEM((D // 2, D), U32),
            pltpu.VMEM((D // 2, D), U32),
            pltpu.VMEM((D // 2, D), U32),
            pltpu.VMEM((F // 2, D), U32),
            pltpu.VMEM((4, 3 * D // 2 + 32, 128), U32),
            pltpu.VMEM((4, D // 2 + 32, 128), U32),
            pltpu.VMEM((D, TL), F32),
            pltpu.VMEM((D // 2, F), U32),
            pltpu.SemaphoreType.DMA((9,)),
            pltpu.SemaphoreType.DMA((NT,)),
            pltpu.SemaphoreType.DMA((NT + 1,)),
            pltpu.SemaphoreType.REGULAR,
        ],
        compiler_params=pltpu.CompilerParams(vmem_limit_bytes=100 * 1024 * 1024),
    )(xt, A_wqkv, A_wo, B_w1, B_w2, B_w3, w4t)
    return out.T.reshape(1, S, D)
```
